```python
import jax
import jax.numpy as jnp

def _softmax(x, axis=-1):
    return jax.nn.softmax(x, axis=axis)
def _gelu(x):
    return jax.nn.gelu(x, approximate=True)
def _silu(x):
    return jax.nn.silu(x)
def _sigmoid(x):
    return jax.nn.sigmoid(x)
def _layernorm(x, axis=-1, eps=1e-5):
    m = jnp.mean(x, axis=axis, keepdims=True)
    v = jnp.var(x, axis=axis, keepdims=True)
    return (x - m) / jnp.sqrt(v + eps)
def _scatter_add(tgt, idx, src, axis=0):
    return tgt.at[idx].add(src)
def _segment_sum(src, seg, n):
    return jax.ops.segment_sum(src, seg, n)
class _Rng:
    def __init__(self, key):
        self._k = key
    def _next(self):
        self._k, sub = jax.random.split(self._k)
        return sub
    def normal(self, shape):
        return jax.random.normal(self._next(), shape, dtype=jnp.bfloat16)
    def randint(self, lo, hi, shape):
        return jax.random.randint(self._next(), shape, lo, hi, dtype=jnp.int32)
    def uniform(self, shape, lo=0.0, hi=1.0):
        return jax.random.uniform(self._next(), shape, jnp.bfloat16, lo, hi)
    def permutation(self, n):
        return jax.random.permutation(self._next(), n)


kernel_name = 'standalone__structured_sparse_n_m__ragged'

def setup_inputs():
    _rng = _Rng(jax.random.key(int.from_bytes(__import__("os").urandom(4), "little")))
    _w = (lambda a: (lambda t: t.astype(jnp.bfloat16) if jnp.issubdtype(t.dtype, jnp.floating) else t)(jnp.asarray(a)))
    B, S, D = 16, 4096, 576
    assert D % 4 == 0, "d_model must be divisible by M=4 for 2:4 sparsity"
    return {
        "x": _w((lambda *s: _rng.normal(s) * 0.05)(B, S, D)),
        "w": _w((lambda *s: _rng.normal(s) * 0.05)(D, D)),
        "b": _w((lambda *s: _rng.normal(s) * 0.05)(D)),
    }

def reference(x, w, b):
    B, S, D = x.shape
    N, M = 2, 4
    G = D // M
    wg = w.reshape(G, M, D)
    mag = jnp.abs(wg)
    order = jnp.argsort(mag, 1)
    thr = jnp.take_along_axis(mag, order[:, M - N:M - N + 1, :], 1)
    mask = (lambda x, dt: x.astype(dt))(mag >= thr, w.dtype)
    wp = (wg * mask).reshape(D, D)
    return jnp.einsum("bsd,df->bsf", x, wp) + b
```

```python
import jax
import jax.numpy as jnp
from jax import lax
import jax.experimental.pallas as pl
import jax.experimental.pallas.tpu as pltpu


def _prune_transposed(w_ref):
    w = w_ref[...].astype(jnp.float32)
    d = w.shape[0]
    mag = jnp.abs(w)
    pos = lax.broadcasted_iota(jnp.int32, w.shape, 0) % 4
    cnt = jnp.zeros(w.shape, jnp.int32)
    for s in (1, 2, 3):
        up = pltpu.roll(mag, s, 0)
        dn = pltpu.roll(mag, d - s, 0)
        cnt = cnt + jnp.where((pos >= s) & (up > mag), 1, 0)
        cnt = cnt + jnp.where((pos + s <= 3) & (dn > mag), 1, 0)
    wp = jnp.where(cnt <= 1, w, 0.0)
    return wp.T


@jax.jit
def pallas_standalone__structured_sparse_n_m__ragged_kernel(
    x: jax.Array,
    w: jax.Array,
    b: jax.Array,
):
    B, S, D = x.shape
    TN = 2048

    def kernel(x_ref, w_ref, b_ref, o_ref, wt_ref):
        @pl.when((pl.program_id(0) == 0) & (pl.program_id(1) == 0))
        def _():
            wt_ref[...] = _prune_transposed(w_ref).astype(jnp.bfloat16)

        acc = jnp.dot(wt_ref[:, :512], x_ref[:512, :], preferred_element_type=jnp.float32)
        acc += jnp.dot(wt_ref[:, 512:], x_ref[512:, :], preferred_element_type=jnp.float32)
        o_ref[...] = (acc + b_ref[...].astype(jnp.float32)).astype(o_ref.dtype)

    xt = jnp.transpose(x, (0, 2, 1))
    out = pl.pallas_call(
        kernel,
        grid=(B, S // TN),
        in_specs=[
            pl.BlockSpec((None, D, TN), lambda i, j: (i, 0, j)),
            pl.BlockSpec((D, D), lambda i, j: (0, 0)),
            pl.BlockSpec((D, 1), lambda i, j: (0, 0)),
        ],
        out_specs=pl.BlockSpec((None, D, TN), lambda i, j: (i, 0, j)),
        out_shape=jax.ShapeDtypeStruct((B, D, S), x.dtype),
        scratch_shapes=[pltpu.VMEM((D, D), jnp.bfloat16)],
        compiler_params=pltpu.CompilerParams(
            dimension_semantics=("arbitrary", "arbitrary"),
            vmem_limit_bytes=100 * 1024 * 1024,
        ),
    )(xt, w, b.reshape(D, 1))
    return jnp.transpose(out, (0, 2, 1))
```

```python
import jax
import jax.numpy as jnp
from jax import lax
import jax.experimental.pallas as pl
import jax.experimental.pallas.tpu as pltpu

F32 = jnp.float32
BF16 = jnp.bfloat16
U32 = jnp.uint32

D = 576
H = D // 2
TN = 512
US = 2 * TN
WN = 256
NX = 10
NO = 9
NT = 17


def _prune(w):
    u = pltpu.bitcast(w, U32).reshape(D // 16, 8, D)
    odd = (lax.broadcasted_iota(jnp.int32, u.shape, 1) & 1) == 1
    p = jnp.where(odd, pltpu.roll(u, 1, 1), pltpu.roll(u, 7, 1))

    def mags(v):
        return (pltpu.bitcast((v << 16) & U32(0x7FFF0000), F32),
                pltpu.bitcast(v & U32(0x7FFF0000), F32))

    a, b = mags(u)
    c, d = mags(p)
    thr = jnp.maximum(jnp.minimum(jnp.maximum(a, b), jnp.maximum(c, d)),
                      jnp.maximum(jnp.minimum(a, b), jnp.minimum(c, d)))
    keep = (jnp.where(a >= thr, U32(0x0000FFFF), U32(0))
            | jnp.where(b >= thr, U32(0xFFFF0000), U32(0)))
    return pltpu.bitcast((u & keep).reshape(D // 2, D), BF16)


def _build_lhs(wt, a_ref):
    a1, a2 = wt[:H], wt[H:]
    lo = lax.broadcasted_iota(jnp.int32, (H, 128), 1) < 64

    def t(a, i):
        return a[:, 128 * i:128 * (i + 1)].astype(F32)

    p11, p12, p21, p22 = t(a1, 0), t(a1, 1), t(a2, 0), t(a2, 1)
    q11, q12, q21, q22 = t(a1, 2), t(a1, 3), t(a2, 2), t(a2, 3)
    r1 = a1[:, 512:].astype(F32)
    r2 = a2[:, 512:].astype(F32)
    r1 = jnp.concatenate([r1, r1], axis=1)
    r2 = jnp.concatenate([r2, r2], axis=1)
    s1, s2, s5, s6, s7 = q11 + q22, q21 + q22, q11 + q12, q21 - q11, q12 - q22
    tiles = [
        p11 + p22, jnp.where(lo, s1, 0.0),
        jnp.where(lo, 0.0, s1),
        p21 + p22, jnp.where(lo, s2, -s2),
        p11, jnp.where(lo, q11, -q22),
        p22, jnp.where(lo, q22, -q11),
        p11 + p12, jnp.where(lo, s5, -s5),
        p21 - p11, jnp.where(lo, s6, r2),
        p12 - p22, jnp.where(lo, s7, r1),
        jnp.where(lo, r2, s6),
        jnp.where(lo, r1, s7),
    ]
    for i, tile in enumerate(tiles):
        a_ref[:, 128 * i:128 * (i + 1)] = pltpu.bitcast(tile.astype(BF16), U32)


def _cols(c0, n):
    if isinstance(c0, int):
        return pl.ds(c0, n)
    return pl.ds(pl.multiple_of(c0, 128), n)


def _unit(a_ref, bias_ref, x_ref, o_ref, c0):
    def x1(r0, r1):
        return x_ref[r0:r1, _cols(c0, TN)]

    def x2(r0, r1):
        return x_ref[r0:r1, _cols(c0 + TN, TN)]

    def add(u, v):
        return (u.astype(F32) + v.astype(F32)).astype(BF16)

    def sub(u, v):
        return (u.astype(F32) - v.astype(F32)).astype(BF16)

    def dot(s0, *rhs):
        rhs = jnp.concatenate(rhs, axis=0)
        lhs = pltpu.bitcast(a_ref[:, 128 * s0:128 * s0 + rhs.shape[0]], BF16)
        return jnp.dot(lhs, rhs, preferred_element_type=F32)

    def bias(half):
        return jnp.concatenate([bias_ref[half * H:(half + 1) * H, :]] * (TN // 128), axis=1)

    def store(fh, th, c):
        o_ref[fh * H:(fh + 1) * H, _cols(c0 + th * TN, TN)] = c.astype(BF16)

    t2 = dot(3, x1(0, 128), x1(256, 320), x2(320, 384))
    c21 = bias(1) + t2
    c22 = bias(1) - t2
    t4 = dot(7, sub(x1(128, 256), x1(0, 128)), sub(x1(384, 512), x1(256, 384)))
    c11 = bias(0) + t4
    c21 = c21 + t4
    c21 = c21 + dot(15, x1(512, 576), add(x1(320, 384), x2(320, 384)))
    q1 = (add(x1(256, 320), x2(384, 448)), add(x2(320, 384), x1(448, 512)))
    t1p = dot(2, *q1)
    c12 = bias(0) + t1p
    store(1, 0, c21 + t1p)
    t5 = dot(9, x2(128, 256), x2(384, 448), x1(448, 512))
    c11 = c11 - t5
    c12 = c12 + t5
    t3 = dot(5, sub(x2(0, 128), x2(128, 256)), sub(x2(256, 384), x2(384, 512)))
    c12 = c12 + t3
    c22 = c22 + t3
    store(0, 1, c12 + dot(16, x2(512, 576), add(x1(448, 512), x2(448, 512))))
    t1 = dot(0, add(x1(0, 128), x2(128, 256)), *q1)
    c11 = c11 + t1
    c22 = c22 + t1
    store(0, 0, c11 + dot(13, add(x1(128, 256), x2(128, 256)),
                          add(x1(384, 448), x2(384, 448)), x1(512, 576)))
    store(1, 1, c22 + dot(11, add(x1(0, 128), x2(0, 128)),
                          add(x1(256, 320), x2(256, 320)), x2(512, 576)))


_PLAN = (0, 0, 0, 0, 0, 0, 0, 3, 2, 2, 2, 2, 1, 1, 1, 1)


def _kernel(x_hbm, w_hbm, b_hbm, o_hbm, xbuf, obuf, wbuf, bbuf, a_ref, bias_ref, tbl,
            xsem, x0sem, osem, wsem):
    nb, _, s_len = x_hbm.shape
    nu = s_len // US
    first = [sum(_PLAN[:s]) for s in range(nb)]
    assert len(_PLAN) == nb and first[-1] + _PLAN[-1] == nb - 1
    assert all(first[s] + _PLAN[s] <= s for s in range(nb))
    assert all(first[s] >= s - NO + 1 for s in range(NO, nb))

    def rd(c, slot):
        return pltpu.make_async_copy(x_hbm.at[c], xbuf.at[slot], xsem.at[slot])

    def rd0(u):
        cs = _cols(u * US, US)
        return pltpu.make_async_copy(x_hbm.at[0, :, cs], xbuf.at[0, :, cs], x0sem.at[u])

    def wr_start(c, slot, c0, n):
        for j in range(n // WN):
            cs = _cols(c0 + j * WN, WN)
            pltpu.make_async_copy(obuf.at[slot, :, cs], o_hbm.at[c, :, cs], osem.at[slot]).start()

    def wr_wait(slot):
        pltpu.make_async_copy(obuf.at[slot], obuf.at[slot], osem.at[slot]).wait()

    def wrap(i, n):
        return jnp.where(i >= n, i - n, i)

    w_copy = pltpu.make_async_copy(w_hbm, wbuf, wsem.at[0])
    b_copy = pltpu.make_async_copy(b_hbm, bbuf, wsem.at[1])
    w_copy.start()
    b_copy.start()
    for u in range(nu):
        rd0(u).start(priority=1)
    for c in range(1, NX):
        rd(c, c).start(priority=1)
    for s in range(nb):
        tbl[0, s] = first[s]
        tbl[1, s] = _PLAN[s]
    b_copy.wait()
    bias_ref[...] = jnp.broadcast_to(bbuf[...].astype(F32).reshape(1, D), (128, D)).T
    w_copy.wait()
    _build_lhs(_prune(wbuf[...]).T, a_ref)

    def first_batch(u, carry):
        rd0(u).wait()
        _unit(a_ref, bias_ref, xbuf.at[0], obuf.at[0], u * US)
        return carry

    lax.fori_loop(0, nu, first_batch, 0)

    def step(s, carry):
        xs = wrap(s, NX)
        os_ = wrap(s, NO)

        @pl.when(s >= NO)
        def _():
            wr_wait(os_)

        rd(s, xs).wait()

        @pl.when(s - 1 + NX < nb)
        def _():
            rd(s - 1 + NX, s - 1).start(priority=1)

        lo = tbl[0, s]
        cnt = tbl[1, s]
        for j in range(max(_PLAN[1:-1])):
            @pl.when(j < cnt)
            def _():
                wr_start(lo + j, wrap(lo + j, NO), 0, s_len)

        for v in range(nu):
            _unit(a_ref, bias_ref, xbuf.at[xs], obuf.at[os_], v * US)
        return carry

    lax.fori_loop(1, nb - 1, step, 0)

    last = nb - 1
    wr_wait(last % NO)
    rd(last, last % NX).wait()
    for c in range(first[last], last):
        wr_start(c, c % NO, 0, s_len)

    def last_batch(u, carry):
        @pl.when(u >= 1)
        def _():
            wr_start(last, last % NO, (u - 1) * US, US)

        _unit(a_ref, bias_ref, xbuf.at[last % NX], obuf.at[last % NO], u * US)
        return carry

    lax.fori_loop(0, nu, last_batch, 0)
    wr_start(last, last % NO, (nu - 1) * US, US)
    for c in range(nb - NO, nb):
        wr_wait(c % NO)


@jax.jit
def pallas_standalone__structured_sparse_n_m__ragged_kernel(
    x: jax.Array,
    w: jax.Array,
    b: jax.Array,
):
    nb, s_len, d = x.shape
    assert d == D and nb == len(_PLAN) and s_len % US == 0
    out_t = pl.pallas_call(
        _kernel,
        in_specs=[pl.BlockSpec(memory_space=pl.ANY)] * 3,
        out_specs=pl.BlockSpec(memory_space=pl.ANY),
        out_shape=jax.ShapeDtypeStruct((nb, D, s_len), x.dtype),
        scratch_shapes=[
            pltpu.VMEM((NX, D, s_len), BF16),
            pltpu.VMEM((NO, D, s_len), BF16),
            pltpu.VMEM((D, D), BF16),
            pltpu.VMEM((D,), BF16),
            pltpu.VMEM((H // 2, NT * 128), U32),
            pltpu.VMEM((D, 128), F32),
            pltpu.SMEM((2, nb), jnp.int32),
            pltpu.SemaphoreType.DMA((NX,)),
            pltpu.SemaphoreType.DMA((s_len // US,)),
            pltpu.SemaphoreType.DMA((NO,)),
            pltpu.SemaphoreType.DMA((2,)),
        ],
        compiler_params=pltpu.CompilerParams(
            vmem_limit_bytes=120 * 1024 * 1024,
            disable_bounds_checks=True,
        ),
    )(jnp.transpose(x, (0, 2, 1)), w, b)
    return jnp.transpose(out_t, (0, 2, 1))
```

```python
import jax
import jax.numpy as jnp
from jax import lax
import jax.experimental.pallas as pl
import jax.experimental.pallas.tpu as pltpu

F32 = jnp.float32
BF16 = jnp.bfloat16
U32 = jnp.uint32

D = 576
H = D // 2
HH = H // 2
TH = 128
TN = 2 * TH
US = 2 * TN
UPB = 4
NFIRST = 4
NX = 10
NO = 10
G0 = 61
RATE = 4
NPAD = 31

_FAST = ("T3", "T4", "T5", "T2")
_SLOT = dict(T1=0, T1p=2, T6=3, T7=5, T6p=7, T7p=8)
_NSLOT = 9
_OUTER = dict(T1=((0, 1), (3, 1)), T1p=((1, 1), (2, 1)), T2=((2, 1), (3, -1)),
              T3=((1, 1), (3, 1)), T4=((0, 1), (2, 1)), T5=((0, -1), (1, 1)),
              T6=((3, 1),), T7=((0, 1),), T6p=((2, 1),), T7p=((1, 1),))
_INNER = {1: ((0, 1), (3, 1)), 2: ((2, 1), (3, -1)), 3: ((1, 1), (3, 1)),
          4: ((0, 1), (2, 1)), 5: ((0, -1), (1, 1)), 6: ((3, 1),), 7: ((0, 1),)}
_ORDER = ("T2", "T3", "T6p", "T4", "T1p", "T7p", "T1", "T5", "T7", "T6")
_INNER_ORDER = (2, 4, 5, 3, 7, 6, 1)


def _prune(w):
    u = pltpu.bitcast(w, U32).reshape(D // 16, 8, D)
    odd = (lax.broadcasted_iota(jnp.int32, u.shape, 1) & 1) == 1
    p = jnp.where(odd, pltpu.roll(u, 1, 1), pltpu.roll(u, 7, 1))

    def mags(v):
        return (pltpu.bitcast((v << 16) & U32(0x7FFF0000), F32),
                pltpu.bitcast(v & U32(0x7FFF0000), F32))

    a, b = mags(u)
    c, d = mags(p)
    thr = jnp.maximum(jnp.minimum(jnp.maximum(a, b), jnp.maximum(c, d)),
                      jnp.maximum(jnp.minimum(a, b), jnp.minimum(c, d)))
    keep = (jnp.where(a >= thr, U32(0x0000FFFF), U32(0))
            | jnp.where(b >= thr, U32(0xFFFF0000), U32(0)))
    return pltpu.bitcast((u & keep).reshape(D // 2, D), BF16)


def _build_lhs(wt, a_ref, a2_ref):
    a1, a2 = wt[:H], wt[H:]
    lo = lax.broadcasted_iota(jnp.int32, (H, 128), 1) < 64

    def t(a, i):
        return a[:, 128 * i:128 * (i + 1)].astype(F32)

    p11, p12, p21, p22 = t(a1, 0), t(a1, 1), t(a2, 0), t(a2, 1)
    q11, q12, q21, q22 = t(a1, 2), t(a1, 3), t(a2, 2), t(a2, 3)
    r1 = a1[:, 512:].astype(F32)
    r2 = a2[:, 512:].astype(F32)
    r1 = jnp.concatenate([r1, r1], axis=1)
    r2 = jnp.concatenate([r2, r2], axis=1)
    s1, s2, s5, s6, s7 = q11 + q22, q21 + q22, q11 + q12, q21 - q11, q12 - q22
    tiles = dict(
        T1=(p11 + p22, jnp.where(lo, s1, 0.0)),
        T1p=(jnp.where(lo, 0.0, s1),),
        T2=(p21 + p22, jnp.where(lo, s2, -s2)),
        T3=(p11, jnp.where(lo, q11, -q22)),
        T4=(p22, jnp.where(lo, q22, -q11)),
        T5=(p11 + p12, jnp.where(lo, s5, -s5)),
        T6=(p21 - p11, jnp.where(lo, s6, r2)),
        T7=(p12 - p22, jnp.where(lo, s7, r1)),
        T6p=(jnp.where(lo, r2, s6),),
        T7p=(jnp.where(lo, r1, s7),),
    )

    def put(ref, i, tile):
        ref[:, 128 * i:128 * (i + 1)] = pltpu.bitcast(tile.astype(BF16), U32)

    for name, tl in tiles.items():
        if name in _FAST:
            l11, l21, l12, l22 = tl[0][:HH], tl[0][HH:], tl[1][:HH], tl[1][HH:]
            ms = (l11 + l22, l21 + l22, l11, l22, l11 + l12, l21 - l11, l12 - l22)
            for i, m in enumerate(ms):
                put(a2_ref, 7 * _FAST.index(name) + i, m)
        else:
            for i, m in enumerate(tl):
                put(a_ref, _SLOT[name] + i, m)


def _one(h, r0, r1):
    return ((1, h, r0, r1),)


def _add(a, b):
    return ((1,) + a, (1,) + b)


def _sub(a, b):
    return ((1,) + a, (-1,) + b)


_Q1 = (_add((0, 256, 320), (1, 384, 448)), _add((1, 320, 384), (0, 448, 512)))
_RHS = dict(
    T1=((_add((0, 0, 128), (1, 128, 256)),), _Q1),
    T1p=(_Q1,),
    T2=((_one(0, 0, 128),), (_one(0, 256, 320), _one(1, 320, 384))),
    T3=((_sub((1, 0, 128), (1, 128, 256)),), (_sub((1, 256, 384), (1, 384, 512)),)),
    T4=((_sub((0, 128, 256), (0, 0, 128)),), (_sub((0, 384, 512), (0, 256, 384)),)),
    T5=((_one(1, 128, 256),), (_one(1, 384, 448), _one(0, 448, 512))),
    T6=((_add((0, 0, 128), (1, 0, 128)),),
        (_add((0, 256, 320), (1, 256, 320)), _one(1, 512, 576))),
    T7=((_add((0, 128, 256), (1, 128, 256)),),
        (_add((0, 384, 448), (1, 384, 448)), _one(0, 512, 576))),
    T6p=((_one(0, 512, 576), _add((0, 320, 384), (1, 320, 384))),),
    T7p=((_one(1, 512, 576), _add((0, 448, 512), (1, 448, 512))),),
)


def _unit(a_ref, a2_ref, bias_ref, x_ref, o_ref, u):
    def rows(pieces, off, n, f32):
        out = []
        for terms in pieces:
            vals = [x_ref[r0:r1, pl.ds(u * US + h * TN + off, n)] for _, h, r0, r1 in terms]
            if len(terms) == 1 and not f32:
                out.append(vals[0])
                continue
            acc = vals[0].astype(F32)
            for (sign, *_), v in zip(terms[1:], vals[1:]):
                acc = acc + v.astype(F32) if sign > 0 else acc - v.astype(F32)
            out.append(acc if f32 else acc.astype(BF16))
        return out[0] if len(out) == 1 else jnp.concatenate(out, axis=0)

    def dot(ref, slot, rhs):
        lhs = pltpu.bitcast(ref[:, 128 * slot:128 * slot + rhs.shape[0]], BF16)
        return jnp.dot(lhs, rhs, preferred_element_type=F32)

    acc = [[None] * 4 for _ in range(4)]
    left = [[4] * 4 for _ in range(4)]

    def accumulate(name, j, val):
        for i, sign in _OUTER[name]:
            r0 = (i // 2) * H + (j // 2) * HH
            base = bias_ref[r0:r0 + HH, :] if acc[i][j] is None else acc[i][j]
            acc[i][j] = base + val if sign > 0 else base - val
            left[i][j] -= 1
            if left[i][j] == 0 and left[i][j ^ 1] == 0:
                band = jnp.concatenate([acc[i][j & 2], acc[i][j | 1]], axis=1)
                o_ref[2 * u + i % 2, r0:r0 + HH, :] = band.astype(BF16)

    for name in _ORDER:
        if name not in _FAST:
            t = dot(a_ref, _SLOT[name], rows(sum(_RHS[name], ()), 0, TN, False))
            for j in range(4):
                accumulate(name, j, t[(j // 2) * HH:(j // 2 + 1) * HH,
                                      (j % 2) * TH:(j % 2 + 1) * TH])
            continue
        k1, k2 = _RHS[name]

        def r(k, j, f32=True):
            return rows(k, j * TH, TH, f32)

        rhs = {1: lambda: (r(k1, 0) + r(k2, 1)).astype(BF16),
               2: lambda: r(k1, 0, False),
               3: lambda: (r(k1, 1) - r(k2, 1)).astype(BF16),
               4: lambda: (r(k2, 0) - r(k1, 0)).astype(BF16),
               5: lambda: r(k2, 1, False),
               6: lambda: (r(k1, 0) + r(k1, 1)).astype(BF16),
               7: lambda: (r(k2, 0) + r(k2, 1)).astype(BF16)}
        quad = [None] * 4
        todo = [4, 2, 2, 4]
        for i in _INNER_ORDER:
            m = dot(a2_ref, 7 * _FAST.index(name) + i - 1, rhs[i]())
            for j, sign in _INNER[i]:
                if quad[j] is None:
                    quad[j] = m if sign > 0 else -m
                else:
                    quad[j] = quad[j] + m if sign > 0 else quad[j] - m
                todo[j] -= 1
                if todo[j] == 0:
                    accumulate(name, j, quad[j])


def _kernel(x_hbm, w_hbm, b_hbm, o_hbm, xbuf, obuf, wbuf, bbuf, a_ref, a2_ref, bias_ref,
            xsem, x0sem, osem, wsem):
    nb, _, s_len = x_hbm.shape
    nu = s_len // US
    npc = s_len // TN
    log_nu = nu.bit_length() - 1
    log_npc = npc.bit_length() - 1
    n_iter = (nb * nu - NFIRST) // UPB

    def issued(g):
        return max(0, min(RATE * (g - G0 + 1), 2 * g))

    assert nu == 1 << log_nu and nu % UPB == 0 and NFIRST % UPB == 0 and NFIRST < nu
    assert NFIRST + n_iter * UPB == nb * nu and NFIRST < G0 and NX <= nb <= 2 * min(NX, NO)
    assert all(issued(c * nu - 1) >= (c - NO + 1) * npc for c in range(NO, nb))

    def wrap(i, n):
        return jnp.where(i >= n, i - n, i)

    def read(c, slot):
        return pltpu.make_async_copy(x_hbm.at[c], xbuf.at[slot], xsem.at[slot])

    def read0(u):
        cols = pl.ds(u * US if isinstance(u, int) else pl.multiple_of(u * US, US), US)
        return pltpu.make_async_copy(x_hbm.at[0, :, cols], xbuf.at[0, :, cols], x0sem.at[u])

    def write_start(q):
        if isinstance(q, int):
            c, j = q // npc, q % npc
            slot, cols = c % NO, pl.ds(j * TN, TN)
        else:
            c, j = lax.shift_right_logical(q, log_npc), lax.bitwise_and(q, npc - 1)
            slot, cols = wrap(c, NO), pl.ds(pl.multiple_of(j * TN, TN), TN)
        pltpu.make_async_copy(obuf.at[slot, j], o_hbm.at[c, :, cols], osem.at[slot]).start(priority=1)

    def write_wait(slot):
        pltpu.make_async_copy(obuf.at[slot], obuf.at[slot], osem.at[slot]).wait()

    def views(xs, os_, v, n):
        return (xbuf.at[xs, :, pl.ds(pl.multiple_of(v * US, n * US), n * US)],
                obuf.at[os_, pl.ds(2 * v, 2 * n)])

    w_copy = pltpu.make_async_copy(w_hbm, wbuf, wsem.at[0])
    b_copy = pltpu.make_async_copy(b_hbm, bbuf, wsem.at[1])
    b_copy.start(priority=1)
    w_copy.start(priority=1)

    @pl.loop(0, nu)
    def _(u):
        read0(u).start(priority=1)

    @pl.loop(1, NX)
    def _(c):
        read(c, c).start(priority=1)

    for k in range(NPAD):
        obuf[NO - 1, k // 72, 8 * (k % 72):8 * (k % 72 + 1), :] = jnp.zeros((8, TN), BF16)

    b_copy.wait()
    bias_ref[...] = jnp.broadcast_to(bbuf[...].astype(F32).reshape(1, D), (TH, D)).T
    w_copy.wait()
    _build_lhs(_prune(wbuf[...]).T, a_ref, a2_ref)

    @pl.loop(0, NFIRST)
    def _(u):
        read0(u).wait()
        _unit(a_ref, a2_ref, bias_ref, *views(0, 0, u, 1), 0)

    for u in range(NFIRST, nu):
        read0(u).wait()

    def body(i, lo):
        g0 = NFIRST + i * UPB
        c = lax.shift_right_logical(g0, log_nu)
        v = lax.bitwise_and(g0, nu - 1)
        xs, os_ = wrap(c, NX), wrap(c, NO)

        @pl.when(jnp.logical_and(v == 0, c >= NO))
        def _():
            write_wait(os_)

        @pl.when(v == 0)
        def _():
            read(c, xs).wait()

        x_ref, o_ref = views(xs, os_, v, UPB)
        for u in range(UPB):
            g = g0 + u
            hi = jnp.maximum(0, jnp.minimum(RATE * (g - G0 + 1), 2 * g))
            for j in range(RATE):
                @pl.when(lo + j < hi)
                def _():
                    write_start(lo + j)
            lo = hi
            _unit(a_ref, a2_ref, bias_ref, x_ref, o_ref, u)

        @pl.when(jnp.logical_and(v == nu - UPB, c + NX < nb))
        def _():
            read(c + NX, xs).start(priority=1)

        return lo

    lax.fori_loop(0, n_iter, body, jnp.int32(0))
    for q in range(issued(nb * nu - 1), nb * npc):
        write_start(q)
    for c in range(nb - NO, nb):
        write_wait(c % NO)


@jax.jit
def pallas_standalone__structured_sparse_n_m__ragged_kernel(
    x: jax.Array,
    w: jax.Array,
    b: jax.Array,
):
    nb, s_len, d = x.shape
    assert d == D and w.shape == (D, D) and b.shape == (D,)
    out_t = pl.pallas_call(
        _kernel,
        in_specs=[pl.BlockSpec(memory_space=pl.ANY)] * 3,
        out_specs=pl.BlockSpec(memory_space=pl.ANY),
        out_shape=jax.ShapeDtypeStruct((nb, D, s_len), x.dtype),
        scratch_shapes=[
            pltpu.VMEM((NX, D, s_len), BF16),
            pltpu.VMEM((NO, s_len // TN, D, TN), BF16),
            pltpu.VMEM((D, D), BF16),
            pltpu.VMEM((D,), BF16),
            pltpu.VMEM((H // 2, _NSLOT * 128), U32),
            pltpu.VMEM((HH // 2, 7 * len(_FAST) * 128), U32),
            pltpu.VMEM((D, TH), F32),
            pltpu.SemaphoreType.DMA((NX,)),
            pltpu.SemaphoreType.DMA((s_len // US,)),
            pltpu.SemaphoreType.DMA((NO,)),
            pltpu.SemaphoreType.DMA((2,)),
        ],
        compiler_params=pltpu.CompilerParams(
            vmem_limit_bytes=120 * 1024 * 1024,
            disable_bounds_checks=True,
        ),
    )(jnp.transpose(x, (0, 2, 1)), w, b)
    return jnp.transpose(out_t, (0, 2, 1))
```

```python
import jax
import jax.numpy as jnp
from jax import lax
import jax.experimental.pallas as pl
import jax.experimental.pallas.tpu as pltpu

F32 = jnp.float32
BF16 = jnp.bfloat16
U32 = jnp.uint32

D = 576
H = D // 2
HH = H // 2
TH = 128
TN = 2 * TH
US = 2 * TN
NX = 10
NO = 10
G0 = 62
RATE = 4
NPAD = 30

_FAST = ("T3", "T4", "T5", "T2")
_SWAP = ("T2", "T5")
_SLOT = dict(T1=0, T1p=2, T6=3, T7=5, T6p=7, T7p=8)
_NSLOT = 9
_OUTER = dict(T1=((0, 1), (3, 1)), T1p=((1, 1), (2, 1)), T2=((2, 1), (3, -1)),
              T3=((1, 1), (3, 1)), T4=((0, 1), (2, 1)), T5=((0, -1), (1, 1)),
              T6=((3, 1),), T7=((0, 1),), T6p=((2, 1),), T7p=((1, 1),))
_INNER = {1: ((0, 1), (3, 1)), 2: ((2, 1), (3, -1)), 3: ((1, 1), (3, 1)),
          4: ((0, 1), (2, 1)), 5: ((0, -1), (1, 1)), 6: ((3, 1),), 7: ((0, 1),)}
_ORDER = ("T2", "T3", "T6p", "T4", "T1p", "T7p", "T1", "T5", "T7", "T6")
_INNER_ORDER = (2, 4, 5, 3, 7, 6, 1)


def _prune(w):
    u = pltpu.bitcast(w, U32).reshape(D // 16, 8, D)
    odd = (lax.broadcasted_iota(jnp.int32, u.shape, 1) & 1) == 1
    p = jnp.where(odd, pltpu.roll(u, 1, 1), pltpu.roll(u, 7, 1))

    def mags(v):
        return (pltpu.bitcast((v << 16) & U32(0x7FFF0000), F32),
                pltpu.bitcast(v & U32(0x7FFF0000), F32))

    a, b = mags(u)
    c, d = mags(p)
    thr = jnp.maximum(jnp.minimum(jnp.maximum(a, b), jnp.maximum(c, d)),
                      jnp.maximum(jnp.minimum(a, b), jnp.minimum(c, d)))
    keep = (jnp.where(a >= thr, U32(0x0000FFFF), U32(0))
            | jnp.where(b >= thr, U32(0xFFFF0000), U32(0)))
    return pltpu.bitcast((u & keep).reshape(D // 2, D), BF16)


def _build_lhs(wt, a_ref, a2_ref):
    a1, a2 = wt[:H], wt[H:]
    lo = lax.broadcasted_iota(jnp.int32, (H, 128), 1) < 64

    def t(a, i):
        return a[:, 128 * i:128 * (i + 1)].astype(F32)

    p11, p12, p21, p22 = t(a1, 0), t(a1, 1), t(a2, 0), t(a2, 1)
    q11, q12, q21, q22 = t(a1, 2), t(a1, 3), t(a2, 2), t(a2, 3)
    r1 = a1[:, 512:].astype(F32)
    r2 = a2[:, 512:].astype(F32)
    r1 = jnp.concatenate([r1, r1], axis=1)
    r2 = jnp.concatenate([r2, r2], axis=1)
    s1, s2, s5, s6, s7 = q11 + q22, q21 + q22, q11 + q12, q21 - q11, q12 - q22
    tiles = dict(
        T1=(p11 + p22, jnp.where(lo, s1, 0.0)),
        T1p=(jnp.where(lo, 0.0, s1),),
        T2=(p21 + p22, jnp.where(lo, s2, -s2)),
        T3=(p11, jnp.where(lo, q11, -q22)),
        T4=(p22, jnp.where(lo, q22, -q11)),
        T5=(p11 + p12, jnp.where(lo, s5, -s5)),
        T6=(p21 - p11, jnp.where(lo, s6, r2)),
        T7=(p12 - p22, jnp.where(lo, s7, r1)),
        T6p=(jnp.where(lo, r2, s6),),
        T7p=(jnp.where(lo, r1, s7),),
    )

    def put(ref, i, tile):
        ref[:, 128 * i:128 * (i + 1)] = pltpu.bitcast(tile.astype(BF16), U32)

    for name, tl in tiles.items():
        if name in _FAST:
            l11, l21, l12, l22 = tl[0][:HH], tl[0][HH:], tl[1][:HH], tl[1][HH:]
            ms = (l11 + l22, l21 + l22, l11, l22, l11 + l12, l21 - l11, l12 - l22)
            for i, m in enumerate(ms):
                put(a2_ref, 7 * _FAST.index(name) + i, m)
        else:
            for i, m in enumerate(tl):
                put(a_ref, _SLOT[name] + i, m)


def _one(h, r0, r1):
    return ((1, h, r0, r1),)


def _add(a, b):
    return ((1,) + a, (1,) + b)


def _sub(a, b):
    return ((1,) + a, (-1,) + b)


_Q1 = (_add((0, 256, 320), (1, 384, 448)), _add((1, 320, 384), (0, 448, 512)))
_RHS = dict(
    T1=((_add((0, 0, 128), (1, 128, 256)),), _Q1),
    T1p=(_Q1,),
    T2=((_one(0, 0, 128),), (_one(0, 256, 320), _one(1, 320, 384))),
    T3=((_sub((1, 0, 128), (1, 128, 256)),), (_sub((1, 256, 384), (1, 384, 512)),)),
    T4=((_sub((0, 128, 256), (0, 0, 128)),), (_sub((0, 384, 512), (0, 256, 384)),)),
    T5=((_one(1, 128, 256),), (_one(1, 384, 448), _one(0, 448, 512))),
    T6=((_add((0, 0, 128), (1, 0, 128)),),
        (_add((0, 256, 320), (1, 256, 320)), _one(1, 512, 576))),
    T7=((_add((0, 128, 256), (1, 128, 256)),),
        (_add((0, 384, 448), (1, 384, 448)), _one(0, 512, 576))),
    T6p=((_one(0, 512, 576), _add((0, 320, 384), (1, 320, 384))),),
    T7p=((_one(1, 512, 576), _add((0, 448, 512), (1, 448, 512))),),
)


def _unit(a_ref, a2_ref, bias_ref, x_ref, o_ref, u):
    def rows(pieces, off, n, f32):
        out = []
        for terms in pieces:
            vals = [x_ref[r0:r1, pl.ds(u * US + h * TN + off, n)] for _, h, r0, r1 in terms]
            if len(terms) == 1 and not f32:
                out.append(vals[0])
                continue
            acc = vals[0].astype(F32)
            for (sign, *_), v in zip(terms[1:], vals[1:]):
                acc = acc + v.astype(F32) if sign > 0 else acc - v.astype(F32)
            out.append(acc if f32 else acc.astype(BF16))
        return out[0] if len(out) == 1 else jnp.concatenate(out, axis=0)

    def dot(ref, slot, rhs):
        lhs = pltpu.bitcast(ref[:, 128 * slot:128 * slot + rhs.shape[0]], BF16)
        return jnp.dot(lhs, rhs, preferred_element_type=F32)

    acc = [[None] * 4 for _ in range(4)]
    left = [[4] * 4 for _ in range(4)]

    def accumulate(name, j, val):
        for i, sign in _OUTER[name]:
            r0 = (i // 2) * H + (j // 2) * HH
            base = bias_ref[r0:r0 + HH, :] if acc[i][j] is None else acc[i][j]
            acc[i][j] = base + val if sign > 0 else base - val
            left[i][j] -= 1
            if left[i][j] == 0 and left[i][j ^ 1] == 0:
                band = jnp.concatenate([acc[i][j & 2], acc[i][j | 1]], axis=1)
                o_ref[2 * u + i % 2, r0:r0 + HH, :] = band.astype(BF16)

    for name in _ORDER:
        if name not in _FAST:
            t = dot(a_ref, _SLOT[name], rows(sum(_RHS[name], ()), 0, TN, False))
            for j in range(4):
                accumulate(name, j, t[(j // 2) * HH:(j // 2 + 1) * HH,
                                      (j % 2) * TH:(j % 2 + 1) * TH])
            continue
        k1, k2 = _RHS[name]
        swap = int(name in _SWAP)

        def r(k, j, f32=True):
            return rows(k, (j ^ swap) * TH, TH, f32)

        rhs = {1: lambda: (r(k1, 0) + r(k2, 1)).astype(BF16),
               2: lambda: r(k1, 0, False),
               3: lambda: (r(k1, 1) - r(k2, 1)).astype(BF16),
               4: lambda: (r(k2, 0) - r(k1, 0)).astype(BF16),
               5: lambda: r(k2, 1, False),
               6: lambda: (r(k1, 0) + r(k1, 1)).astype(BF16),
               7: lambda: (r(k2, 0) + r(k2, 1)).astype(BF16)}
        quad = [None] * 4
        todo = [4, 2, 2, 4]
        for i in _INNER_ORDER:
            m = dot(a2_ref, 7 * _FAST.index(name) + i - 1, rhs[i]())
            for j, sign in _INNER[i]:
                if quad[j] is None:
                    quad[j] = m if sign > 0 else -m
                else:
                    quad[j] = quad[j] + m if sign > 0 else quad[j] - m
                todo[j] -= 1
                if todo[j] == 0:
                    accumulate(name, j ^ swap, quad[j])


def _kernel(x_hbm, w_hbm, b_hbm, o_hbm, xbuf, obuf, wbuf, bbuf, a_ref, a2_ref, bias_ref,
            xsem, x0sem, osem, wsem):
    nb, _, s_len = x_hbm.shape
    nu = s_len // US
    npc = s_len // TN
    log_npc = npc.bit_length() - 1

    def issued(g):
        return max(0, min(RATE * (g - G0 + 1), 2 * g))

    assert npc == 1 << log_npc and nu <= G0 and max(NX, NO) < nb <= 2 * min(NX, NO)
    assert all(issued(c * nu - 1) >= (c - NO + 1) * npc for c in range(NO, nb))

    def wrap(i, n):
        return jnp.where(i >= n, i - n, i)

    def read(c, slot):
        return pltpu.make_async_copy(x_hbm.at[c], xbuf.at[slot], xsem.at[slot])

    def read0(u):
        cols = pl.ds(pl.multiple_of(u * US, US), US)
        return pltpu.make_async_copy(x_hbm.at[0, :, cols], xbuf.at[0, :, cols], x0sem.at[u])

    def write_start(q):
        if isinstance(q, int):
            c, j = q // npc, q % npc
            slot, cols = c % NO, pl.ds(j * TN, TN)
        else:
            c, j = lax.shift_right_logical(q, log_npc), lax.bitwise_and(q, npc - 1)
            slot, cols = wrap(c, NO), pl.ds(pl.multiple_of(j * TN, TN), TN)
        pltpu.make_async_copy(obuf.at[slot, j], o_hbm.at[c, :, cols], osem.at[slot]).start(priority=1)

    def write_wait(slot):
        pltpu.make_async_copy(obuf.at[slot], obuf.at[slot], osem.at[slot]).wait()

    w_copy = pltpu.make_async_copy(w_hbm, wbuf, wsem.at[0])
    b_copy = pltpu.make_async_copy(b_hbm, bbuf, wsem.at[1])
    b_copy.start(priority=1)
    w_copy.start(priority=1)

    @pl.loop(0, nu)
    def _(u):
        read0(u).start(priority=1)

    @pl.loop(1, NX)
    def _(c):
        read(c, c).start(priority=1)

    for k in range(NPAD):
        obuf[NO - 1, 0, 8 * k:8 * (k + 1), :] = jnp.zeros((8, TN), BF16)

    b_copy.wait()
    bias_ref[...] = jnp.broadcast_to(bbuf[...].astype(F32).reshape(1, D), (TH, D)).T
    w_copy.wait()
    _build_lhs(_prune(wbuf[...]).T, a_ref, a2_ref)

    @pl.loop(0, nu)
    def _(u):
        read0(u).wait()
        _unit(a_ref, a2_ref, bias_ref,
              xbuf.at[0, :, pl.ds(pl.multiple_of(u * US, US), US)],
              obuf.at[0, pl.ds(2 * u, 2)], 0)

    read(NX, 0).start(priority=1)

    def batch(c, lo):
        xs, os_ = wrap(c, NX), wrap(c, NO)

        @pl.when(c >= NO)
        def _():
            write_wait(os_)

        read(c, xs).wait()
        for u in range(nu):
            g = c * nu + u
            hi = jnp.maximum(0, jnp.minimum(RATE * (g - G0 + 1), 2 * g))
            for j in range(RATE):
                @pl.when(lo + j < hi)
                def _():
                    write_start(lo + j)
            lo = hi
            _unit(a_ref, a2_ref, bias_ref, xbuf.at[xs], obuf.at[os_], u)

        @pl.when(c + NX < nb)
        def _():
            read(c + NX, xs).start(priority=1)

        return lo

    lax.fori_loop(1, nb, batch, jnp.int32(0))
    for q in range(issued(nb * nu - 1), nb * npc):
        write_start(q)
    for c in range(nb - NO, nb):
        write_wait(c % NO)


@jax.jit
def pallas_standalone__structured_sparse_n_m__ragged_kernel(
    x: jax.Array,
    w: jax.Array,
    b: jax.Array,
):
    nb, s_len, d = x.shape
    assert d == D and w.shape == (D, D) and b.shape == (D,)
    out_t = pl.pallas_call(
        _kernel,
        in_specs=[pl.BlockSpec(memory_space=pl.ANY)] * 3,
        out_specs=pl.BlockSpec(memory_space=pl.ANY),
        out_shape=jax.ShapeDtypeStruct((nb, D, s_len), x.dtype),
        scratch_shapes=[
            pltpu.VMEM((NX, D, s_len), BF16),
            pltpu.VMEM((NO, s_len // TN, D, TN), BF16),
            pltpu.VMEM((D, D), BF16),
            pltpu.VMEM((D,), BF16),
            pltpu.VMEM((H // 2, _NSLOT * 128), U32),
            pltpu.VMEM((HH // 2, 7 * len(_FAST) * 128), U32),
            pltpu.VMEM((D, TH), F32),
            pltpu.SemaphoreType.DMA((NX,)),
            pltpu.SemaphoreType.DMA((s_len // US,)),
            pltpu.SemaphoreType.DMA((NO,)),
            pltpu.SemaphoreType.DMA((2,)),
        ],
        compiler_params=pltpu.CompilerParams(
            vmem_limit_bytes=120 * 1024 * 1024,
            disable_bounds_checks=True,
        ),
    )(jnp.transpose(x, (0, 2, 1)), w, b)
    return jnp.transpose(out_t, (0, 2, 1))
```

```python
import jax
import jax.numpy as jnp
from jax import lax
import jax.experimental.pallas as pl
import jax.experimental.pallas.tpu as pltpu

F32 = jnp.float32
BF16 = jnp.bfloat16
U32 = jnp.uint32

D = 576
H = D // 2
HH = H // 2
TH = 128
TN = 2 * TH
US = 2 * TN
NSLAB = 9
SLAB = D // NSLAB
NRG = SLAB // 8
WCOL = 2 * US
NX = 10
NO = 10
G0 = 63
RATE = 8
C_COL = 14

_FAST = ("T3", "T4", "T5", "T2")
_SWAP = ("T2", "T5")
_SLOT = dict(T1=0, T1p=2, T6=3, T7=5, T6p=7, T7p=8)
_NSLOT = 9
_OUTER = dict(T1=((0, 1), (3, 1)), T1p=((1, 1), (2, 1)), T2=((2, 1), (3, -1)),
              T3=((1, 1), (3, 1)), T4=((0, 1), (2, 1)), T5=((0, -1), (1, 1)),
              T6=((3, 1),), T7=((0, 1),), T6p=((2, 1),), T7p=((1, 1),))
_INNER = {1: ((0, 1), (3, 1)), 2: ((2, 1), (3, -1)), 3: ((1, 1), (3, 1)),
          4: ((0, 1), (2, 1)), 5: ((0, -1), (1, 1)), 6: ((3, 1),), 7: ((0, 1),)}
_ORDER = ("T2", "T3", "T6p", "T4", "T1p", "T7p", "T1", "T5", "T7", "T6")
_INNER_ORDER = (2, 4, 5, 3, 7, 6, 1)


def _prune(w):
    u = pltpu.bitcast(w, U32).reshape(D // 16, 8, D)
    odd = (lax.broadcasted_iota(jnp.int32, u.shape, 1) & 1) == 1
    p = jnp.where(odd, pltpu.roll(u, 1, 1), pltpu.roll(u, 7, 1))

    def mags(v):
        return (pltpu.bitcast((v << 16) & U32(0x7FFF0000), F32),
                pltpu.bitcast(v & U32(0x7FFF0000), F32))

    a, b = mags(u)
    c, d = mags(p)
    thr = jnp.maximum(jnp.minimum(jnp.maximum(a, b), jnp.maximum(c, d)),
                      jnp.maximum(jnp.minimum(a, b), jnp.minimum(c, d)))
    keep = (jnp.where(a >= thr, U32(0x0000FFFF), U32(0))
            | jnp.where(b >= thr, U32(0xFFFF0000), U32(0)))
    return pltpu.bitcast((u & keep).reshape(D // 2, D), BF16)


def _build_lhs(wt, a_ref, a2_ref):
    a1, a2 = wt[:H], wt[H:]
    lo = lax.broadcasted_iota(jnp.int32, (H, 128), 1) < 64

    def t(a, i):
        return a[:, 128 * i:128 * (i + 1)].astype(F32)

    p11, p12, p21, p22 = t(a1, 0), t(a1, 1), t(a2, 0), t(a2, 1)
    q11, q12, q21, q22 = t(a1, 2), t(a1, 3), t(a2, 2), t(a2, 3)
    r1 = a1[:, 512:].astype(F32)
    r2 = a2[:, 512:].astype(F32)
    r1 = jnp.concatenate([r1, r1], axis=1)
    r2 = jnp.concatenate([r2, r2], axis=1)
    s1, s2, s5, s6, s7 = q11 + q22, q21 + q22, q11 + q12, q21 - q11, q12 - q22
    tiles = dict(
        T1=(p11 + p22, jnp.where(lo, s1, 0.0)),
        T1p=(jnp.where(lo, 0.0, s1),),
        T2=(p21 + p22, jnp.where(lo, s2, -s2)),
        T3=(p11, jnp.where(lo, q11, -q22)),
        T4=(p22, jnp.where(lo, q22, -q11)),
        T5=(p11 + p12, jnp.where(lo, s5, -s5)),
        T6=(p21 - p11, jnp.where(lo, s6, r2)),
        T7=(p12 - p22, jnp.where(lo, s7, r1)),
        T6p=(jnp.where(lo, r2, s6),),
        T7p=(jnp.where(lo, r1, s7),),
    )

    def put(ref, i, tile):
        ref[:, 128 * i:128 * (i + 1)] = pltpu.bitcast(tile.astype(BF16), U32)

    for name, tl in tiles.items():
        if name in _FAST:
            l11, l21, l12, l22 = tl[0][:HH], tl[0][HH:], tl[1][:HH], tl[1][HH:]
            ms = (l11 + l22, l21 + l22, l11, l22, l11 + l12, l21 - l11, l12 - l22)
            for i, m in enumerate(ms):
                put(a2_ref, 7 * _FAST.index(name) + i, m)
        else:
            for i, m in enumerate(tl):
                put(a_ref, _SLOT[name] + i, m)


def _one(h, r0, r1):
    return ((1, h, r0, r1),)


def _add(a, b):
    return ((1,) + a, (1,) + b)


def _sub(a, b):
    return ((1,) + a, (-1,) + b)


_Q1 = (_add((0, 256, 320), (1, 384, 448)), _add((1, 320, 384), (0, 448, 512)))
_RHS = dict(
    T1=((_add((0, 0, 128), (1, 128, 256)),), _Q1),
    T1p=(_Q1,),
    T2=((_one(0, 0, 128),), (_one(0, 256, 320), _one(1, 320, 384))),
    T3=((_sub((1, 0, 128), (1, 128, 256)),), (_sub((1, 256, 384), (1, 384, 512)),)),
    T4=((_sub((0, 128, 256), (0, 0, 128)),), (_sub((0, 384, 512), (0, 256, 384)),)),
    T5=((_one(1, 128, 256),), (_one(1, 384, 448), _one(0, 448, 512))),
    T6=((_add((0, 0, 128), (1, 0, 128)),),
        (_add((0, 256, 320), (1, 256, 320)), _one(1, 512, 576))),
    T7=((_add((0, 128, 256), (1, 128, 256)),),
        (_add((0, 384, 448), (1, 384, 448)), _one(0, 512, 576))),
    T6p=((_one(0, 512, 576), _add((0, 320, 384), (1, 320, 384))),),
    T7p=((_one(1, 512, 576), _add((0, 448, 512), (1, 448, 512))),),
)


def _unit(a_ref, a2_ref, bias_ref, x_ref, o_ref, u, on_block=None):
    def rows(pieces, off, n, f32):
        out = []
        for terms in pieces:
            vals = [x_ref[r0:r1, pl.ds(u * US + h * TN + off, n)] for _, h, r0, r1 in terms]
            if len(terms) == 1 and not f32:
                out.append(vals[0])
                continue
            acc = vals[0].astype(F32)
            for (sign, *_), v in zip(terms[1:], vals[1:]):
                acc = acc + v.astype(F32) if sign > 0 else acc - v.astype(F32)
            out.append(acc if f32 else acc.astype(BF16))
        return out[0] if len(out) == 1 else jnp.concatenate(out, axis=0)

    def dot(ref, slot, rhs):
        lhs = pltpu.bitcast(ref[:, 128 * slot:128 * slot + rhs.shape[0]], BF16)
        return jnp.dot(lhs, rhs, preferred_element_type=F32)

    acc = [[None] * 4 for _ in range(4)]
    left = [[4] * 4 for _ in range(4)]

    def accumulate(name, j, val):
        for i, sign in _OUTER[name]:
            r0 = (i // 2) * H + (j // 2) * HH
            base = bias_ref[r0:r0 + HH, :] if acc[i][j] is None else acc[i][j]
            acc[i][j] = base + val if sign > 0 else base - val
            left[i][j] -= 1
            if left[i][j] == 0 and left[i][j ^ 1] == 0:
                band = jnp.concatenate([acc[i][j & 2], acc[i][j | 1]], axis=1).astype(BF16)
                cols = pl.ds(u * US + (i % 2) * TN, TN)
                for g in range(r0 // SLAB, (r0 + HH - 1) // SLAB + 1):
                    lo, hi = max(r0, g * SLAB), min(r0 + HH, (g + 1) * SLAB)
                    o_ref[g, lo - g * SLAB:hi - g * SLAB, cols] = band[lo - r0:hi - r0]
                if on_block is not None and not any(left[i]):
                    on_block(i)

    for name in _ORDER:
        if name not in _FAST:
            t = dot(a_ref, _SLOT[name], rows(sum(_RHS[name], ()), 0, TN, False))
            for j in range(4):
                accumulate(name, j, t[(j // 2) * HH:(j // 2 + 1) * HH,
                                      (j % 2) * TH:(j % 2 + 1) * TH])
            continue
        k1, k2 = _RHS[name]
        swap = int(name in _SWAP)

        def r(k, j, f32=True):
            return rows(k, (j ^ swap) * TH, TH, f32)

        rhs = {1: lambda: (r(k1, 0) + r(k2, 1)).astype(BF16),
               2: lambda: r(k1, 0, False),
               3: lambda: (r(k1, 1) - r(k2, 1)).astype(BF16),
               4: lambda: (r(k2, 0) - r(k1, 0)).astype(BF16),
               5: lambda: r(k2, 1, False),
               6: lambda: (r(k1, 0) + r(k1, 1)).astype(BF16),
               7: lambda: (r(k2, 0) + r(k2, 1)).astype(BF16)}
        quad = [None] * 4
        todo = [4, 2, 2, 4]
        for i in _INNER_ORDER:
            m = dot(a2_ref, 7 * _FAST.index(name) + i - 1, rhs[i]())
            for j, sign in _INNER[i]:
                if quad[j] is None:
                    quad[j] = m if sign > 0 else -m
                else:
                    quad[j] = quad[j] + m if sign > 0 else quad[j] - m
                todo[j] -= 1
                if todo[j] == 0:
                    accumulate(name, j ^ swap, quad[j])


def _kernel(x_hbm, w_hbm, b_hbm, o_hbm, xbuf, obuf, wbuf, bbuf, a_ref, a2_ref, bias_ref,
            xsem, x0sem, osem, wsem):
    nb, _, s_len = x_hbm.shape
    nu = s_len // US
    ncg = s_len // WCOL
    npc = NRG * ncg
    n_reg = nb * npc - NRG
    last, half = nb - 1, nu // 2

    def log2(n):
        assert n & (n - 1) == 0
        return n.bit_length() - 1

    def ready(c, u):
        return npc * c + (c >= C_COL) * (NRG * (u // 2))

    assert 2 * nu <= G0 and nb % 2 == 0 and NX + 2 <= nb <= 2 * min(NX, NO) and NX % 2 == 0
    issued = 0
    for c in range(2, nb):
        if c % 2 == 0:
            assert issued >= (c + 2 - NO) * npc
        for u in range(nu):
            if c * nu + u >= G0:
                issued = min(issued + RATE, ready(c, u))
    assert issued == n_reg

    def wrap(i, n):
        return jnp.where(i >= n, i - n, i)

    def unit_cols(v, n):
        return pl.ds(pl.multiple_of(v * US, n * US), n * US)

    def read(c, slot):
        return pltpu.make_async_copy(x_hbm.at[c], xbuf.at[slot], xsem.at[slot])

    def read0(u):
        cols = unit_cols(u, 1)
        return pltpu.make_async_copy(x_hbm.at[0, :, cols], xbuf.at[0, :, cols], x0sem.at[u])

    def write(c, slot, slabs, rows, cols):
        pltpu.make_async_copy(obuf.at[slot, slabs, rows, cols], o_hbm.at[c, slabs, rows, cols],
                              osem.at[slot]).start(priority=1)

    def write_piece(q):
        c = lax.shift_right_logical(q, log2(npc))
        by_col = c >= C_COL
        r = jnp.where(by_col, lax.bitwise_and(q, NRG - 1),
                      lax.bitwise_and(lax.shift_right_logical(q, log2(ncg)), NRG - 1))
        n = jnp.where(by_col, lax.shift_right_logical(q, log2(NRG)), q)
        write(c, wrap(c, NO), slice(None), pl.ds(pl.multiple_of(8 * r, 8), 8),
              pl.ds(pl.multiple_of(lax.bitwise_and(n, ncg - 1) * WCOL, WCOL), WCOL))

    def write_second_last_unit():
        for r in range(NRG):
            write(last, last % NO, slice(None), pl.ds(8 * r, 8), pl.ds((nu - 2) * US, US))

    def write_last_block(i):
        cols = pl.ds((nu - 1) * US + (i % 2) * TN, TN)
        mid = H // SLAB
        write(last, last % NO, pl.ds((i // 2) * (mid + 1), mid), slice(None), cols)
        write(last, last % NO, pl.ds(mid, 1), pl.ds((i // 2) * (SLAB // 2), SLAB // 2), cols)

    def write_wait(slot):
        pltpu.make_async_copy(obuf.at[slot], obuf.at[slot], osem.at[slot]).wait()

    def units(xs, os_, v, n):
        cols = unit_cols(v, n)
        for u in range(n):
            _unit(a_ref, a2_ref, bias_ref, xbuf.at[xs, :, cols], obuf.at[os_, :, :, cols], u)

    w_copy = pltpu.make_async_copy(w_hbm, wbuf, wsem.at[0])
    b_copy = pltpu.make_async_copy(b_hbm, bbuf, wsem.at[1])
    b_copy.start(priority=1)
    w_copy.start(priority=1)

    @pl.loop(0, nu)
    def _(u):
        read0(u).start(priority=1)

    @pl.loop(1, NX)
    def _(c):
        read(c, c).start(priority=1)

    b_copy.wait()
    bias_ref[...] = jnp.broadcast_to(bbuf[...].astype(F32).reshape(1, D), (TH, D)).T
    w_copy.wait()
    _build_lhs(_prune(wbuf[...]).T, a_ref, a2_ref)

    @pl.loop(0, half)
    def _(u):
        read0(u).wait()
        units(0, 0, u, 1)

    @pl.loop(1, 4)
    def _(i):
        c, v = lax.shift_right_logical(i, 1), lax.bitwise_and(i, 1)

        @pl.when(i == 1)
        def _():
            for u in range(half, nu):
                read0(u).wait()

        @pl.when(i == 2)
        def _():
            read(1, 1).wait()

        units(c, c, v * half, half)

        @pl.when(v == 1)
        def _():
            read(c + NX, c).start(priority=1)

    def batch_pair(i, lo):
        pair = (2 * i, 2 * i + 1)
        for c in pair:
            @pl.when(c >= NO)
            def _():
                write_wait(wrap(c, NO))

            read(c, wrap(c, NX)).wait()

        for c in pair:
            for u in range(nu):
                more = npc * c + jnp.where(c >= C_COL, NRG * (u // 2), 0)
                hi = jnp.where(c * nu + u >= G0, jnp.minimum(lo + RATE, more), 0)
                for j in range(RATE):
                    @pl.when(lo + j < hi)
                    def _():
                        write_piece(lo + j)
                lo = hi
                on_block = None
                if c is pair[1] and u == nu - 1:
                    pl.when(c == last)(write_second_last_unit)

                    def on_block(blk):
                        pl.when(c == last)(lambda: write_last_block(blk))

                _unit(a_ref, a2_ref, bias_ref, xbuf.at[wrap(c, NX)], obuf.at[wrap(c, NO)], u,
                      on_block)

        for c in pair:
            @pl.when(c + NX < nb)
            def _():
                read(c + NX, wrap(c, NX)).start(priority=1)

        return lo

    lax.fori_loop(1, nb // 2, batch_pair, jnp.int32(0))
    for slot in range(NO):
        write_wait(slot)


@jax.jit
def pallas_standalone__structured_sparse_n_m__ragged_kernel(
    x: jax.Array,
    w: jax.Array,
    b: jax.Array,
):
    nb, s_len, d = x.shape
    assert d == D and w.shape == (D, D) and b.shape == (D,)
    out_t = pl.pallas_call(
        _kernel,
        in_specs=[pl.BlockSpec(memory_space=pl.ANY)] * 3,
        out_specs=pl.BlockSpec(memory_space=pl.ANY),
        out_shape=jax.ShapeDtypeStruct((nb, NSLAB, SLAB, s_len), x.dtype),
        scratch_shapes=[
            pltpu.VMEM((NX, D, s_len), BF16),
            pltpu.VMEM((NO, NSLAB, SLAB, s_len), BF16),
            pltpu.VMEM((D, D), BF16),
            pltpu.VMEM((D,), BF16),
            pltpu.VMEM((H // 2, _NSLOT * 128), U32),
            pltpu.VMEM((HH // 2, 7 * len(_FAST) * 128), U32),
            pltpu.VMEM((D, TH), F32),
            pltpu.SemaphoreType.DMA((NX,)),
            pltpu.SemaphoreType.DMA((s_len // US,)),
            pltpu.SemaphoreType.DMA((NO,)),
            pltpu.SemaphoreType.DMA((2,)),
        ],
        compiler_params=pltpu.CompilerParams(
            vmem_limit_bytes=120 * 1024 * 1024,
            disable_bounds_checks=True,
        ),
    )(jnp.transpose(x, (0, 2, 1)), w, b)
    return jnp.transpose(out_t.reshape(nb, D, s_len), (0, 2, 1))
```
